```python
import os as _os
_os.environ.setdefault("JAX_PLATFORMS", "cpu")
import jax
import jax.numpy as jnp

def _softmax(x, axis=-1):
    return jax.nn.softmax(x, axis=axis)
def _gelu(x):
    return jax.nn.gelu(x, approximate=True)
def _silu(x):
    return jax.nn.silu(x)
def _sigmoid(x):
    return jax.nn.sigmoid(x)
def _layernorm(x, axis=-1, eps=1e-5):
    m = jnp.mean(x, axis=axis, keepdims=True)
    v = jnp.var(x, axis=axis, keepdims=True)
    return (x - m) / jnp.sqrt(v + eps)
def _scatter_add(tgt, idx, src, axis=0):
    return tgt.at[idx].add(src)
def _segment_sum(src, seg, n):
    return jax.ops.segment_sum(src, seg, n)
class _Rng:
    def __init__(self, key):
        self._k = key
    def _next(self):
        self._k, sub = jax.random.split(self._k)
        return sub
    def normal(self, shape):
        return jax.random.normal(self._next(), shape, dtype=jnp.bfloat16)
    def randint(self, lo, hi, shape):
        return jax.random.randint(self._next(), shape, lo, hi, dtype=jnp.int32)
    def uniform(self, shape, lo=0.0, hi=1.0):
        return jax.random.uniform(self._next(), shape, jnp.bfloat16, lo, hi)
    def permutation(self, n):
        return jax.random.permutation(self._next(), n)


kernel_name = 'sequential_preLN__linear_attn_block__glu_gated_reglu__prompt'

def setup_inputs():
    _rng = _Rng(jax.random.key(int.from_bytes(__import__("os").urandom(4), "little")))
    _w = (lambda a: (lambda t: t.astype(jnp.bfloat16) if jnp.issubdtype(t.dtype, jnp.floating) else t)(jnp.asarray(a)))
    def _A_setup():
        B, S, D = 1, 2048, 640
        return {
            "x": _w((lambda *s: _rng.normal(s) * 0.05)(B, S, D)),
            "wqkv": _w((lambda *s: _rng.normal(s) * 0.05)(D, 3 * D)),
            "wo": _w((lambda *s: _rng.normal(s) * 0.05)(D, D)),
        }
    _A_in = _A_setup()

    def _B_setup():
        B, S, D, F = 1, 2048, 640, 1536
        return {
            "x": _w((lambda *s: _rng.normal(s) * 0.05)(B, S, D)),
            "W_gate": _w((lambda *s: _rng.normal(s) * 0.05)(D, F) * (2.0 / D) ** 0.5),
            "W_up": _w((lambda *s: _rng.normal(s) * 0.05)(D, F) * (2.0 / D) ** 0.5),
            "W_down": _w((lambda *s: _rng.normal(s) * 0.05)(F, D) * (1.0 / F) ** 0.5),
        }
    _B_in = _B_setup()

    return {
        "A_x": _A_in["x"],
        "A_wqkv": _A_in["wqkv"],
        "A_wo": _A_in["wo"],
        "B_x": _B_in["x"],
        "B_W_gate": _B_in["W_gate"],
        "B_W_up": _B_in["W_up"],
        "B_W_down": _B_in["W_down"],
    }

def reference(A_x, A_wqkv, A_wo, B_x, B_W_gate, B_W_up, B_W_down):
    def _A_ref(x, wqkv, wo):
        B, S, D = x.shape
        H = 32; Dh = D // H
        qkv = (lambda x, *d: x.transpose(*d))((x @ wqkv).reshape(B, S, 3, H, Dh), 2, 0, 3, 1, 4)
        q, k, v = qkv[0], qkv[1], qkv[2]
        phi = lambda t: jnp.where(t > 0, t + 1, jnp.exp(t)) + 1e-6
        pq, pk = phi(q), phi(k)
        kv = jnp.einsum("bhsd,bhse->bhde", pk, v)
        z = jnp.einsum("bhsd->bhd", pk)
        num = jnp.einsum("bhqd,bhde->bhqe", pq, kv)
        den = jnp.einsum("bhqd,bhd->bhq", pq, z)[..., None] + 1e-6
        o = num / den
        return (lambda x, *d: x.transpose(*d))(o, 0, 2, 1, 3).reshape(B, S, D) @ wo

    def _B_ref(x, W_gate, W_up, W_down):
        gate = jnp.einsum("bsd,df->bsf", x, W_gate)
        up = jnp.einsum("bsd,df->bsf", x, W_up)
        gate = gate * (lambda x, dt: x.astype(dt))(gate > 0, gate.dtype)
        h = gate * up
        return jnp.einsum("bsf,fd->bsd", h, W_down)

    x = A_x
    h = x + _A_ref(_layernorm(x, axis=-1), A_wqkv, A_wo)
    h2 = h + _B_ref(_layernorm(h, axis=-1), B_W_gate, B_W_up, B_W_down)
    return h2
```

```python
import functools
import numpy as np
import jax
import jax.numpy as jnp
from jax import lax
import jax.experimental.pallas as pl
import jax.experimental.pallas.tpu as pltpu

S, D, H, DH, F = 2048, 640, 32, 20, 1536
T1 = 512
T2 = 512
FC = 512


def _ln(x):
    m = jnp.mean(x, axis=-1, keepdims=True)
    xc = x - m
    v = jnp.mean(xc * xc, axis=-1, keepdims=True)
    return xc * lax.rsqrt(v + 1e-5)


def _phi(t):
    return jnp.where(t > 0, t + 1.0, jnp.exp(t)) + 1e-6


def _kernel(x_hbm, wqkv_hbm, wo_hbm, wg_hbm, wu_hbm, wd_hbm, o_hbm,
            x_v, xn_v, wq_v, wk_v, wv_v, wo_v, wg_v, wu_v, wd_v,
            wqp_v, mp_v, f32_v, o_v, sem_x, sem_w, sem_o):
    n1, n2 = S // T1, S // T2

    def x_copy(i):
        return pltpu.make_async_copy(x_hbm.at[pl.ds(i * T1, T1)], x_v.at[pl.ds(i * T1, T1)], sem_x.at[i])

    w_copies = dict(
        k=pltpu.make_async_copy(wqkv_hbm.at[:, pl.ds(D, D)], wk_v, sem_w.at[0]),
        q=pltpu.make_async_copy(wqkv_hbm.at[:, pl.ds(0, D)], wq_v, sem_w.at[1]),
        v=pltpu.make_async_copy(wqkv_hbm.at[:, pl.ds(2 * D, D)], wv_v, sem_w.at[2]),
        o=pltpu.make_async_copy(wo_hbm, wo_v, sem_w.at[3]),
        g=pltpu.make_async_copy(wg_hbm, wg_v, sem_w.at[4]),
        u=pltpu.make_async_copy(wu_hbm, wu_v, sem_w.at[5]),
        d=pltpu.make_async_copy(wd_hbm, wd_v, sem_w.at[6]),
    )
    x_copy(0).start()
    w_copies['k'].start()
    for i in range(1, n1):
        x_copy(i).start()
    for n in 'qvogud':
        w_copies[n].start()

    w_copies['k'].wait()

    def p1(i, zacc):
        x_copy(i).wait()
        r0 = pl.multiple_of(i * T1, T1)
        x = x_v[pl.ds(r0, T1), :].astype(jnp.float32)
        xn = _ln(x).astype(jnp.bfloat16)
        xn_v[pl.ds(r0, T1), :] = xn
        k = jnp.dot(xn, wk_v[...], preferred_element_type=jnp.float32)
        pk = _phi(k)
        zacc = zacc + jnp.sum(pk.reshape(T1 // 8, 8, D), axis=0)
        p = lax.dot_general(pk.astype(jnp.bfloat16), xn, (((0,), (0,)), ((), ())),
                            preferred_element_type=jnp.float32)

        @pl.when(i == 0)
        def _():
            for j in range(5):
                f32_v[j] = p[:, j * 128:(j + 1) * 128]

        @pl.when(i > 0)
        def _():
            for j in range(5):
                f32_v[j] += p[:, j * 128:(j + 1) * 128]
        return zacc

    zacc = lax.fori_loop(0, n1, p1, jnp.zeros((8, D), jnp.float32))

    w_copies['v'].wait()
    w_copies['o'].wait()
    kv = jnp.dot(jnp.concatenate([f32_v[j] for j in range(5)], axis=1).astype(jnp.bfloat16), wv_v[...], preferred_element_type=jnp.float32)
    row_h = lax.broadcasted_iota(jnp.int32, (D, D), 0) // DH
    col_h = lax.broadcasted_iota(jnp.int32, (D, D), 1) // DH
    kv = jnp.where(row_h == col_h, kv, 0.0).astype(jnp.bfloat16)
    m = jnp.dot(kv, wo_v[...], preferred_element_type=jnp.float32)
    for j in range(5):
        f32_v[j] = m[:, j * 128:(j + 1) * 128]
    for d in range(DH):
        for j in range(5):
            mp_v[d * H:(d + 1) * H, j * 128:(j + 1) * 128] = f32_v[j, pl.ds(d, H, stride=DH), :].astype(jnp.bfloat16)
    zfull = jnp.concatenate([zacc, jnp.zeros((120, D), jnp.float32)], axis=0)
    f32_v[0] = zfull.T
    zp = jnp.concatenate([f32_v[0, pl.ds(d, H, stride=DH), :] for d in range(DH)], axis=0)
    zrow = jnp.sum(zp.T, axis=0, keepdims=True)
    w_copies['q'].wait()
    wqt = wq_v[...].astype(jnp.float32).T
    for j in range(5):
        f32_v[j] = wqt[:, j * 128:(j + 1) * 128]
    for d in range(DH):
        for j in range(5):
            wqp_v[d * H:(d + 1) * H, j * 128:(j + 1) * 128] = f32_v[j, pl.ds(d, H, stride=DH), :].astype(jnp.bfloat16)

    w_copies['g'].wait()
    w_copies['u'].wait()
    w_copies['d'].wait()

    def o_copy(i, slot):
        return pltpu.make_async_copy(o_v.at[slot], o_hbm.at[pl.ds(i * T2, T2)], sem_o.at[slot])

    def p2(i, c):
        slot = i % 2
        r0 = pl.multiple_of(i * T2, T2)
        xn = xn_v[pl.ds(r0, T2), :]
        q = lax.dot_general(xn, wqp_v[...], (((1,), (1,)), ((), ())), preferred_element_type=jnp.float32)
        pq = _phi(q)
        t = pq * zrow
        den = t[:, 0:128] + t[:, 128:256] + t[:, 256:384] + t[:, 384:512] + t[:, 512:640]
        den = den + pltpu.roll(den, 64, 1)
        den = den + pltpu.roll(den, 32, 1)
        r = 1.0 / (den + 1e-6)
        pqn = jnp.concatenate([pq[:, j * 128:(j + 1) * 128] * r for j in range(5)], axis=1)
        attn = jnp.dot(pqn.astype(jnp.bfloat16), mp_v[...], preferred_element_type=jnp.float32)
        h = x_v[pl.ds(r0, T2), :].astype(jnp.float32) + attn
        hn = _ln(h).astype(jnp.bfloat16)
        acc = h
        for c0 in range(0, F, FC):
            g = jnp.dot(hn, wg_v[:, c0:c0 + FC], preferred_element_type=jnp.float32)
            u = jnp.dot(hn, wu_v[:, c0:c0 + FC], preferred_element_type=jnp.float32)
            a = (jnp.where(g > 0, g, 0.0) * u).astype(jnp.bfloat16)
            acc = acc + jnp.dot(a, wd_v[c0:c0 + FC, :], preferred_element_type=jnp.float32)

        @pl.when(i >= 2)
        def _():
            o_copy(i - 2, slot).wait()
        o_v[slot] = acc.astype(jnp.bfloat16)
        o_copy(i, slot).start()
        return c

    lax.fori_loop(0, n2, p2, 0)
    o_copy(n2 - 2, (n2 - 2) % 2).wait()
    o_copy(n2 - 1, (n2 - 1) % 2).wait()


@jax.jit
def pallas_sequential_preLN__linear_attn_block__glu_gated_reglu__prompt_kernel(A_x, A_wqkv, A_wo, B_x, B_W_gate, B_W_up, B_W_down):
    x = A_x.reshape(S, D)
    bf = jnp.bfloat16
    any_spec = pl.BlockSpec(memory_space=pl.ANY)
    out = pl.pallas_call(
        _kernel,
        out_shape=jax.ShapeDtypeStruct((S, D), A_x.dtype),
        in_specs=[any_spec] * 6,
        out_specs=any_spec,
        scratch_shapes=[
            pltpu.VMEM((S, D), bf), pltpu.VMEM((S, D), bf),
            pltpu.VMEM((D, D), bf), pltpu.VMEM((D, D), bf), pltpu.VMEM((D, D), bf), pltpu.VMEM((D, D), bf),
            pltpu.VMEM((D, F), bf), pltpu.VMEM((D, F), bf), pltpu.VMEM((F, D), bf),
            pltpu.VMEM((D, D), bf), pltpu.VMEM((D, D), bf), pltpu.VMEM((5, D, 128), jnp.float32),
            pltpu.VMEM((2, T2, D), bf),
            pltpu.SemaphoreType.DMA((S // T1,)), pltpu.SemaphoreType.DMA((7,)), pltpu.SemaphoreType.DMA((2,)),
        ],
        compiler_params=pltpu.CompilerParams(vmem_limit_bytes=100 * 1024 * 1024),
    )(x, A_wqkv, A_wo, B_W_gate, B_W_up, B_W_down)
    return out.reshape(A_x.shape)
```

```python
import functools
import numpy as np
import jax
import jax.numpy as jnp
from jax import lax
import jax.experimental.pallas as pl
import jax.experimental.pallas.tpu as pltpu

S, D, H, DH, F = 2048, 640, 32, 20, 1536
T = 512
FC = 512
T1S = [256, 256, 512, 512, 512]
T2S = [512, 512, 512, 384, 128]
KCH = 1
O1 = [sum(T1S[:i]) for i in range(len(T1S))]
O2 = [sum(T2S[:i]) for i in range(len(T2S))]
N1, N2 = len(T1S), len(T2S)
bf = jnp.bfloat16
f32 = jnp.float32


def _ln(x):
    m = jnp.mean(x, axis=-1, keepdims=True)
    xc = x - m
    v = jnp.mean(xc * xc, axis=-1, keepdims=True)
    return xc * lax.rsqrt(v + 1e-5)


def _phi(t):
    return jnp.where(t > 0, t + 1.0, jnp.exp(t)) + 1e-6


def _dot(a, b):
    return jnp.dot(a, b, preferred_element_type=f32)


def _dot_nt(a, b):
    return lax.dot_general(a, b, (((1,), (1,)), ((), ())), preferred_element_type=f32)


def _dot_p(a, b):
    return jnp.dot(a, b, preferred_element_type=f32)


def _dot_kv(a, b):
    return jnp.dot(a, b, preferred_element_type=f32)


def _dot_m(a, b):
    return jnp.dot(a, b, preferred_element_type=f32)


def _dot_attn(a, b):
    return jnp.dot(a, b, preferred_element_type=f32)


def _dot_g(a, b):
    return jnp.dot(a, b, preferred_element_type=f32)


def _dot_u(a, b):
    return jnp.dot(a, b, preferred_element_type=f32)


def _dot_d(a, b):
    return jnp.dot(a, b, preferred_element_type=f32)


def _dot_k(a, b):
    return lax.dot_general(a, b, (((1,), (1,)), ((), ())), preferred_element_type=f32)


def _dot_q(a, b):
    return lax.dot_general(a, b, (((1,), (1,)), ((), ())), preferred_element_type=f32)


def _kernel(x_hbm, wqkv_hbm, wo_hbm, wg_hbm, wu_hbm, wd_hbm, o_hbm,
            x_v, xn_v, wq_v, wk_v, wv_v, wo_v, wg_v, wu_v, wd_v,
            wkt_v, wqp_v, mp_v, f32_v, o_v, sem_x, sem_w, sem_o, sem_k):

    def x_copy(i):
        return pltpu.make_async_copy(x_hbm.at[pl.ds(O1[i], T1S[i])], x_v.at[pl.ds(O1[i], T1S[i])], sem_x.at[i])

    def o_copy(i):
        return pltpu.make_async_copy(o_v.at[pl.ds(O2[i], T2S[i])], o_hbm.at[pl.ds(O2[i], T2S[i])], sem_o.at[i])

    w = dict(
        q=pltpu.make_async_copy(wqkv_hbm.at[:, pl.ds(0, D)], wq_v, sem_w.at[1]),
        v=pltpu.make_async_copy(wqkv_hbm.at[:, pl.ds(2 * D, D)], wv_v, sem_w.at[2]),
        o=pltpu.make_async_copy(wo_hbm, wo_v, sem_w.at[3]),
        g=pltpu.make_async_copy(wg_hbm, wg_v, sem_w.at[4]),
        u=pltpu.make_async_copy(wu_hbm, wu_v, sem_w.at[5]),
        d=pltpu.make_async_copy(wd_hbm, wd_v, sem_w.at[6]),
    )
    KR = D // KCH

    def k_copy(c):
        return pltpu.make_async_copy(wqkv_hbm.at[pl.ds(c * KR, KR), pl.ds(D, D)], wk_v.at[pl.ds(c * KR, KR)], sem_k.at[c])

    def KT(c):
        wkt_v[:, c * KR:(c + 1) * KR] = wk_v[c * KR:(c + 1) * KR, :].astype(f32).T.astype(bf)

    xs, xn = {}, {}

    def LN1(i):
        xn[i] = _ln(x_v[O1[i]:O1[i] + T1S[i], :].astype(f32)).astype(bf)
        xn_v[O1[i]:O1[i] + T1S[i], :] = xn[i]

    pkt = {}
    st = dict(z=None, p=None)

    def K(i):
        if i == 0:
            pk = _phi(_dot(xn[i], wk_v[...])).T
        else:
            pk = _phi(_dot_k(wkt_v[...], xn[i]))
        zs = pk[:, 0:128]
        for j in range(1, T1S[i] // 128):
            zs = zs + pk[:, j * 128:(j + 1) * 128]
        st['z'] = zs if st['z'] is None else st['z'] + zs
        pkt[i] = pk.astype(bf)

    def Pm(i):
        p = _dot_p(pkt[i], xn[i])
        st['p'] = p if st['p'] is None else st['p'] + p

    def perm_rows(val, dst):
        for j in range(5):
            f32_v[j] = val[:, j * 128:(j + 1) * 128]
        for d in range(DH):
            for j in range(5):
                dst[d * H:(d + 1) * H, j * 128:(j + 1) * 128] = f32_v[j, pl.ds(d, H, stride=DH), :].astype(bf)

    def WQ():
        perm_rows(wq_v[...].astype(f32).T, wqp_v)

    pq = {}

    def Q(i):
        pq[i] = _phi(_dot_q(xn_v[O2[i]:O2[i] + T2S[i], :], wqp_v[...]))

    def KVM():
        p = st['p'].astype(bf)
        kvs = []
        for i in range(5):
            c0, c1 = max(0, i - 1) * 128, min(5, i + 2) * 128
            kv = _dot_kv(p[i * 128:(i + 1) * 128, :], wv_v[:, c0:c1])
            rh = (lax.broadcasted_iota(jnp.int32, kv.shape, 0) + i * 128) // DH
            ch = (lax.broadcasted_iota(jnp.int32, kv.shape, 1) + c0) // DH
            kvs.append(jnp.where(rh == ch, kv, 0.0).astype(bf))
        st['kv'] = kvs

    def M():
        ms = []
        for i in range(5):
            c0, c1 = max(0, i - 1) * 128, min(5, i + 2) * 128
            ms.append(_dot_m(st['kv'][i], wo_v[c0:c1, :]))
        perm_rows(jnp.concatenate(ms, axis=0), mp_v)
        f32_v[0] = st['z']
        zp = jnp.concatenate([f32_v[0, pl.ds(d, H, stride=DH), :] for d in range(DH)], axis=0)
        st['zrow'] = jnp.sum(zp.T, axis=0, keepdims=True)

    hs, hn = {}, {}

    def A(i):
        t = pq[i] * st['zrow']
        den = t[:, 0:128] + t[:, 128:256] + t[:, 256:384] + t[:, 384:512] + t[:, 512:640]
        den = den + pltpu.roll(den, 64, 1)
        den = den + pltpu.roll(den, 32, 1)
        r = 1.0 / (den + 1e-6)
        pqn = jnp.concatenate([pq[i][:, j * 128:(j + 1) * 128] * r for j in range(5)], axis=1)
        hs[i] = x_v[O2[i]:O2[i] + T2S[i], :].astype(f32) + _dot_attn(pqn.astype(bf), mp_v[...])
        hn[i] = _ln(hs[i]).astype(bf)

    def Fc(i, c0):
        g = _dot_g(hn[i], wg_v[:, c0:c0 + FC])
        u = _dot_u(hn[i], wu_v[:, c0:c0 + FC])
        a = (jnp.where(g > 0, g, 0.0) * u).astype(bf)
        hs[i] = hs[i] + _dot_d(a, wd_v[c0:c0 + FC, :])

    def Fo(i):
        for c0 in range(0, F, FC):
            Fc(i, c0)
        o_v[O2[i]:O2[i] + T2S[i], :] = hs[i].astype(bf)
        o_copy(i).start()

    x_copy(0).start()
    for c in range(KCH):
        k_copy(c).start()
    x_copy(0).wait()
    x_copy(1).start()
    LN1(0)
    for c in range(KCH):
        k_copy(c).wait()
    x_copy(1).wait()
    x_copy(2).start()
    K(0)
    for c in range(KCH):
        KT(c)
    x_copy(3).start()
    LN1(1)
    K(1)
    Pm(0)
    x_copy(2).wait()
    x_copy(4).start()
    w['q'].start()
    w['v'].start()
    w['o'].start()
    Pm(1)
    x_copy(3).wait()
    w['g'].start()
    w['u'].start()
    w['d'].start()
    LN1(2)
    K(2)
    LN1(3)
    K(3)
    Pm(2)
    x_copy(4).wait()
    w['q'].wait()
    w['v'].wait()
    w['o'].wait()
    Pm(3)
    LN1(4)
    K(4)
    WQ()
    Pm(4)
    Q(0)
    KVM()
    Q(1)
    M()
    Q(2)
    w['g'].wait()
    w['u'].wait()
    w['d'].wait()
    Q(3)
    Q(4)
    A(0)
    A(1)
    Fo(0)
    A(2)
    Fo(1)
    A(3)
    Fo(2)
    A(4)
    Fo(3)
    Fo(4)
    for i in range(N2):
        o_copy(i).wait()


@jax.jit
def pallas_sequential_preLN__linear_attn_block__glu_gated_reglu__prompt_kernel(A_x, A_wqkv, A_wo, B_x, B_W_gate, B_W_up, B_W_down):
    x = A_x.reshape(S, D)
    any_spec = pl.BlockSpec(memory_space=pl.ANY)
    out = pl.pallas_call(
        _kernel,
        out_shape=jax.ShapeDtypeStruct((S, D), A_x.dtype),
        in_specs=[any_spec] * 6,
        out_specs=any_spec,
        scratch_shapes=[
            pltpu.VMEM((S, D), bf), pltpu.VMEM((S, D), bf),
            pltpu.VMEM((D, D), bf), pltpu.VMEM((D, D), bf), pltpu.VMEM((D, D), bf), pltpu.VMEM((D, D), bf),
            pltpu.VMEM((D, F), bf), pltpu.VMEM((D, F), bf), pltpu.VMEM((F, D), bf),
            pltpu.VMEM((D, D), bf), pltpu.VMEM((D, D), bf), pltpu.VMEM((D, D), bf), pltpu.VMEM((5, D, 128), f32),
            pltpu.VMEM((S, D), bf),
            pltpu.SemaphoreType.DMA((N1,)), pltpu.SemaphoreType.DMA((7,)), pltpu.SemaphoreType.DMA((N2,)), pltpu.SemaphoreType.DMA((KCH,)),
        ],
        compiler_params=pltpu.CompilerParams(vmem_limit_bytes=110 * 1024 * 1024),
    )(x, A_wqkv, A_wo, B_W_gate, B_W_up, B_W_down)
    return out.reshape(A_x.shape)
```
